```python
import os as _os
_os.environ.setdefault("JAX_PLATFORMS", "cpu")
import jax
import jax.numpy as jnp

def _softmax(x, axis=-1):
    return jax.nn.softmax(x, axis=axis)
def _gelu(x):
    return jax.nn.gelu(x, approximate=True)
def _silu(x):
    return jax.nn.silu(x)
def _sigmoid(x):
    return jax.nn.sigmoid(x)
def _layernorm(x, axis=-1, eps=1e-5):
    m = jnp.mean(x, axis=axis, keepdims=True)
    v = jnp.var(x, axis=axis, keepdims=True)
    return (x - m) / jnp.sqrt(v + eps)
def _scatter_add(tgt, idx, src, axis=0):
    return tgt.at[idx].add(src)
def _segment_sum(src, seg, n):
    return jax.ops.segment_sum(src, seg, n)
class _Rng:
    def __init__(self, key):
        self._k = key
    def _next(self):
        self._k, sub = jax.random.split(self._k)
        return sub
    def normal(self, shape):
        return jax.random.normal(self._next(), shape, dtype=jnp.bfloat16)
    def randint(self, lo, hi, shape):
        return jax.random.randint(self._next(), shape, lo, hi, dtype=jnp.int32)
    def uniform(self, shape, lo=0.0, hi=1.0):
        return jax.random.uniform(self._next(), shape, jnp.bfloat16, lo, hi)
    def permutation(self, n):
        return jax.random.permutation(self._next(), n)


kernel_name = 'gated_mix__grouped_kv_mqa__ssm_conv_s5__prompt'

def setup_inputs():
    _rng = _Rng(jax.random.key(int.from_bytes(__import__("os").urandom(4), "little")))
    _w = (lambda a: (lambda t: t.astype(jnp.bfloat16) if jnp.issubdtype(t.dtype, jnp.floating) else t)(jnp.asarray(a)))
    def _A_setup():
        B, S, D, H = 1, 2048, 512, 32
        Dh = D // H
        return {
            "x": _w((lambda *s: _rng.normal(s) * 0.05)(B, S, D)),
            "wq": _w((lambda *s: _rng.normal(s) * 1.6)(D, H * Dh)),
            "wk": _w((lambda *s: _rng.normal(s) * 1.6)(D, Dh)),
            "wv": _w((lambda *s: _rng.normal(s) * 0.05)(D, Dh)),
            "wo": _w((lambda *s: _rng.normal(s) * 0.05)(H * Dh, D)),
        }
    _A_in = _A_setup()

    def _B_setup():
        B, S, D = 1, 2048, 512
        P = D
        Lambda_re = -0.5 * jnp.exp((lambda *s: _rng.normal(s) * 0.4)(P))
        Lambda_im = (lambda *s: _rng.normal(s) * 0.4)(P) * 1.0
        B_re = (lambda *s: _rng.normal(s) * 0.4)(P, D) * (D ** -0.5)
        B_im = (lambda *s: _rng.normal(s) * 0.4)(P, D) * (D ** -0.5)
        C_re = (lambda *s: _rng.normal(s) * 0.4)(D, P) * (P ** -0.5)
        C_im = (lambda *s: _rng.normal(s) * 0.4)(D, P) * (P ** -0.5)
        log_dt = (lambda *s: _rng.normal(s) * 0.4)(P) * 0.3 - 2.0
        Dskip = (lambda *s: _rng.normal(s) * 0.4)(D)
        return {
            "x": _w((lambda *s: _rng.normal(s) * 0.05)(B, S, D)),
            "Lambda_re": _w(Lambda_re),
            "Lambda_im": _w(Lambda_im),
            "B_re": _w(B_re),
            "B_im": _w(B_im),
            "C_re": _w(C_re),
            "C_im": _w(C_im),
            "log_dt": _w(log_dt),
            "Dskip": _w(Dskip),
        }
    _B_in = _B_setup()

    return {
        "A_x": _A_in["x"],
        "A_wq": _A_in["wq"],
        "A_wk": _A_in["wk"],
        "A_wv": _A_in["wv"],
        "A_wo": _A_in["wo"],
        "B_x": _B_in["x"],
        "B_Lambda_re": _B_in["Lambda_re"],
        "B_Lambda_im": _B_in["Lambda_im"],
        "B_B_re": _B_in["B_re"],
        "B_B_im": _B_in["B_im"],
        "B_C_re": _B_in["C_re"],
        "B_C_im": _B_in["C_im"],
        "B_log_dt": _B_in["log_dt"],
        "B_Dskip": _B_in["Dskip"],
        "gate_w": _w((lambda *s: _rng.normal(s) * 0.05)(512) * 16.0),
    }

def reference(A_x, A_wq, A_wk, A_wv, A_wo, B_x, B_Lambda_re, B_Lambda_im, B_B_re, B_B_im, B_C_re, B_C_im, B_log_dt, B_Dskip, gate_w):
    def _A_ref(x, wq, wk, wv, wo):
        B, S, D = x.shape
        H = 32
        Dh = D // H
        q = (lambda x, *d: x.transpose(*d))((x @ wq).reshape(B, S, H, Dh), 0, 2, 1, 3)
        k = x @ wk
        v = x @ wv
        scores = jnp.einsum("bhqd,bkd->bhqk", q, k) * (Dh ** -0.5)
        p = _softmax(scores, axis=-1)
        o = jnp.einsum("bhqk,bkd->bhqd", p, v)
        return (lambda x, *d: x.transpose(*d))(o, 0, 2, 1, 3).reshape(B, S, H * Dh) @ wo

    def _B_ref(x, Lambda_re, Lambda_im, B_re, B_im, C_re, C_im, log_dt, Dskip):
        Bsz, L, H = x.shape
        Lam = Lambda_re + 1j * Lambda_im
        Bmat = B_re + 1j * B_im
        Cmat = C_re + 1j * C_im
        dt = jnp.exp(log_dt)
        Lam_bar = jnp.exp(dt * Lam)
        B_bar = ((Lam_bar - 1.0) / Lam)[:, None] * Bmat
        Bu = jnp.einsum("bld,pd->blp", x + 0j, B_bar)
        h = jnp.zeros_like(Bu[:, 0, :])
        hs = []
        for t in range(L):
            h = Lam_bar[None, :] * h + Bu[:, t, :]
            hs.append(h)
        hseq = jnp.stack(hs, 1)
        y = 2.0 * jnp.einsum("blp,dp->bld", hseq, Cmat).real + x * Dskip[None, None, :]
        return y

    x = A_x
    g = _sigmoid((x * gate_w).sum(-1, keepdims=True))
    a = _A_ref(x, A_wq, A_wk, A_wv, A_wo)
    b = _B_ref(x, B_Lambda_re, B_Lambda_im, B_B_re, B_B_im, B_C_re, B_C_im, B_log_dt, B_Dskip)
    return g * a + (1 - g) * b
```

```python
import functools

import jax
import jax.numpy as jnp
from jax import lax
import jax.experimental.pallas as pl
import jax.experimental.pallas.tpu as pltpu

S = 2048
D = 512
H = 32
DH = 16
P = 512
CN = 512
NQ = S // CN
RT = 128
NR = S // RT
NSEG = 8
SEGLEN = S // NSEG
NLT = P // 128
RB = 256

F32 = jnp.float32
BF16 = jnp.bfloat16


def _dot(a, b, ca, cb):
    return lax.dot_general(a, b, (((ca,), (cb,)), ((), ())), preferred_element_type=F32)


def _cmul(ar, ai, br, bi):
    return ar * br - ai * bi, ar * bi + ai * br


def _kernel(x_ref, wq_ref, wk_ref, wv_ref, wo_ref, lre_ref, lim_ref, bre_ref, bim_ref,
            cre_ref, cim_ref, ldt_ref, dsk_ref, gw_ref,
            out_ref,
            qT, kS, vT, oT, s0, s1, m0, m1, bur, bui, bbuf, gbuf):
    qb = pl.program_id(0)

    def attn_step(sa, ma, ha, qba, sb, mb, hb, qbb, do_b=True):
        cola = pl.ds(pl.multiple_of(qba * CN, CN), CN)
        q = qT[pl.ds(pl.multiple_of(ha * DH, DH), DH), cola]
        m8 = jnp.full((8, CN), -jnp.inf, F32)
        if do_b:
            colb = pl.ds(pl.multiple_of(qbb * CN, CN), CN)
            m = jnp.max(mb[...], axis=0, keepdims=True)
            l8 = jnp.zeros((8, CN), F32)
            acc = jnp.zeros((DH, CN), F32)
        for r in range(NR):
            rows = slice(r * RT, (r + 1) * RT)
            if do_b:
                st = sb[rows, :]
            s = _dot(kS[rows, :], q, 1, 0)
            sa[rows, :] = s
            m8 = jnp.maximum(m8, jnp.max(s.reshape(RT // 8, 8, CN), axis=0))
            if do_b:
                p = jnp.exp(st - m)
                l8 = l8 + jnp.sum(p.reshape(RT // 8, 8, CN), axis=0)
                acc = acc + _dot(vT[:, rows], p.astype(BF16), 1, 0)
        ma[...] = m8
        if do_b:
            l = jnp.sum(l8, axis=0, keepdims=True)
            oT[pl.ds(pl.multiple_of(hb * DH, DH), DH), colb] = (acc / l).astype(BF16)

    @pl.when(qb == 0)
    def _prologue():
        x = x_ref[...]
        qT[...] = (_dot(wq_ref[...], x, 0, 1) * (DH ** -0.5)).astype(BF16)
        kS[...] = _dot(x, wk_ref[...], 1, 0).astype(BF16)
        vT[...] = _dot(wv_ref[...], x, 0, 1).astype(BF16)
        gw = gw_ref[...].astype(F32)
        for rb in range(S // RB):
            rows = slice(rb * RB, (rb + 1) * RB)
            gl = jnp.sum(x_ref[rows, :].astype(F32) * gw, axis=-1, keepdims=True)
            gbuf[rows, :] = jnp.broadcast_to(jax.nn.sigmoid(gl), (RB, 128))

        lre = lre_ref[...].astype(F32)
        lim = lim_ref[...].astype(F32)
        dt = jnp.exp(ldt_ref[...].astype(F32))
        zr = dt * lre
        zi = dt * lim
        ez = jnp.exp(zr)
        lbr = ez * jnp.cos(zi)
        lbi = ez * jnp.sin(zi)
        den = lre * lre + lim * lim
        nr = lbr - 1.0
        cr = (nr * lre + lbi * lim) / den
        ci = (lbi * lre - nr * lim) / den
        cre = cre_ref[...].astype(F32)
        cim = cim_ref[...].astype(F32)
        cpr = cre * cr - cim * ci
        cpi = cre * ci + cim * cr
        wy = jnp.concatenate([(2.0 * cpr).astype(BF16), (-2.0 * cpi).astype(BF16)], axis=1)

        for rb in range(S // RB):
            rows = slice(rb * RB, (rb + 1) * RB)
            xb = x_ref[rows, :]
            bur[rows, :] = _dot(xb, bre_ref[...], 1, 1)
            bui[rows, :] = _dot(xb, bim_ref[...], 1, 1)

        sub = lax.broadcasted_iota(jnp.int32, (8, 128), 0)
        tabs = []
        for j in range(NLT):
            cl = slice(j * 128, (j + 1) * 128)
            p1r = jnp.broadcast_to(lbr[:, cl], (8, 128))
            p1i = jnp.broadcast_to(lbi[:, cl], (8, 128))
            p2r, p2i = _cmul(p1r, p1i, p1r, p1i)
            p4r, p4i = _cmul(p2r, p2i, p2r, p2i)
            lev = tuple((d, jnp.where(sub >= d, pr, 0.0), jnp.where(sub >= d, pi, 0.0))
                        for d, pr, pi in ((1, p1r, p1i), (2, p2r, p2i), (4, p4r, p4i)))
            wr = jnp.where(sub == 0, p1r, 0.0)
            wi = jnp.where(sub == 0, p1i, 0.0)
            ar, ai = p1r, p1i
            for t in range(1, 8):
                ar, ai = _cmul(ar, ai, p1r, p1i)
                wr = jnp.where(sub == t, ar, wr)
                wi = jnp.where(sub == t, ai, wi)
            tabs.append((lev, wr, wi))

        def scan_block(b, carry):
            rows = pl.ds(pl.multiple_of(b * 8, 8), 8)
            new = []
            for j in range(NLT):
                cl = slice(j * 128, (j + 1) * 128)
                ur = bur[rows, cl]
                ui = bui[rows, cl]
                lev, wr, wi = tabs[j]
                for d, a_r, a_i in lev:
                    sr = pltpu.roll(ur, d, 0)
                    si = pltpu.roll(ui, d, 0)
                    ur, ui = ur + (a_r * sr - a_i * si), ui + (a_r * si + a_i * sr)
                c_r, c_i = carry[2 * j], carry[2 * j + 1]
                ur, ui = ur + (wr * c_r - wi * c_i), ui + (wr * c_i + wi * c_r)
                bur[rows, cl] = ur
                bui[rows, cl] = ui
                new += [jnp.broadcast_to(ur[7:8, :], (8, 128)), jnp.broadcast_to(ui[7:8, :], (8, 128))]
            return tuple(new)

        lax.fori_loop(0, S // 8, scan_block, tuple(jnp.zeros((8, 128), F32) for _ in range(2 * NLT)),
                      unroll=2)

        dsk = dsk_ref[...].astype(F32)
        for rb in range(S // RB):
            rows = slice(rb * RB, (rb + 1) * RB)
            hb_ = jnp.concatenate([bur[rows, :].astype(BF16), bui[rows, :].astype(BF16)], axis=1)
            bbuf[rows, :] = _dot(hb_, wy, 1, 1) + x_ref[rows, :].astype(F32) * dsk

        attn_step(s0, m0, 0, 0, None, None, None, None, do_b=False)

    trip1 = jnp.minimum(qb, 0) + 1

    def one(sa, ma, ha, qba, sb, mb, hb, qbb):
        def body(_, c):
            attn_step(sa, ma, ha, qba, sb, mb, hb, qbb)
            return c
        lax.fori_loop(0, trip1, body, 0)

    def pair(i, _):
        h0 = 2 * i
        one(s1, m1, h0 + 1, qb, s0, m0, h0, qb)
        last = h0 + 2 >= H
        h_n = jnp.where(last, 0, h0 + 2)
        qb_n = jnp.minimum(jnp.where(last, qb + 1, qb), NQ - 1)
        one(s0, m0, h_n, qb_n, s1, m1, h0 + 1, qb)
        return 0

    lax.fori_loop(0, H // 2, pair, 0)

    col = pl.ds(pl.multiple_of(qb * CN, CN), CN)
    a = _dot(oT[:, col], wo_ref[...], 0, 0)
    g = gbuf[col, :]
    g = jnp.concatenate([g] * (D // 128), axis=1)
    out_ref[...] = g * a + (1.0 - g) * bbuf[col, :]


@jax.jit
def pallas_gated_mix__grouped_kv_mqa__ssm_conv_s5__prompt_kernel(
    A_x: jax.Array,
    A_wq: jax.Array,
    A_wk: jax.Array,
    A_wv: jax.Array,
    A_wo: jax.Array,
    B_x: jax.Array,
    B_Lambda_re: jax.Array,
    B_Lambda_im: jax.Array,
    B_B_re: jax.Array,
    B_B_im: jax.Array,
    B_C_re: jax.Array,
    B_C_im: jax.Array,
    B_log_dt: jax.Array,
    B_Dskip: jax.Array,
    gate_w: jax.Array,
):
    del B_x
    x = A_x.reshape(S, D)
    row = lambda v: v.reshape(1, -1)
    ins = (x, A_wq, A_wk, A_wv, A_wo, row(B_Lambda_re), row(B_Lambda_im), B_B_re, B_B_im,
           B_C_re, B_C_im, row(B_log_dt), row(B_Dskip), row(gate_w))
    full = lambda a: pl.BlockSpec(a.shape, lambda qb: (0, 0))
    out = pl.pallas_call(
        _kernel,
        grid=(NQ,),
        in_specs=[full(a) for a in ins],
        out_specs=pl.BlockSpec((CN, D), lambda qb: (qb, 0)),
        out_shape=jax.ShapeDtypeStruct((S, D), F32),
        scratch_shapes=[
            pltpu.VMEM((H * DH, S), BF16),
            pltpu.VMEM((S, DH), BF16),
            pltpu.VMEM((DH, S), BF16),
            pltpu.VMEM((H * DH, S), BF16),
            pltpu.VMEM((S, CN), F32),
            pltpu.VMEM((S, CN), F32),
            pltpu.VMEM((8, CN), F32),
            pltpu.VMEM((8, CN), F32),
            pltpu.VMEM((S, P), F32),
            pltpu.VMEM((S, P), F32),
            pltpu.VMEM((S, D), F32),
            pltpu.VMEM((S, 128), F32),
        ],
        compiler_params=pltpu.CompilerParams(
            dimension_semantics=("arbitrary",),
            vmem_limit_bytes=100 * 1024 * 1024,
        ),
    )(*ins)
    return out.reshape(1, S, D)
```

```python
import jax
import jax.numpy as jnp
from jax import lax
import jax.experimental.pallas as pl
import jax.experimental.pallas.tpu as pltpu

S = 2048
D = 512
H = 32
DH = 16
P = 512
CN = 512
NQ = S // CN
RT = 128
NR = S // RT
NLT = P // 128
RB = 256
SPB = (S // 8) // (NQ * H)
SCAN_AT = (4, 11)

F32 = jnp.float32
BF16 = jnp.bfloat16


def _dot(a, b, ca, cb):
    return lax.dot_general(a, b, (((ca,), (cb,)), ((), ())), preferred_element_type=F32)


def _cmul(ar, ai, br, bi):
    return ar * br - ai * bi, ar * bi + ai * br


def _row(ref):
    return ref[...].reshape(1, -1).astype(F32)


def _kernel(x_ref, wq_ref, wkv_ref, wo_ref, lre_ref, lim_ref, bre_ref, bim_ref,
            cre_ref, cim_ref, ldt_ref, dsk_ref, gw_ref,
            out_ref,
            qT, kS, vT, oT, s0, s1, m0, m1, bur, bui, gbuf, l8r, tab, hc, wyb):
    qb = pl.program_id(0)

    def scan_blocks(b0, n):
        carry = [hc[i] for i in range(2 * NLT)]
        for bb in range(n):
            rows = pl.ds(pl.multiple_of((b0 + bb) * 8, 8), 8)
            for j in range(NLT):
                cl = slice(j * 128, (j + 1) * 128)
                ur = bur[rows, cl]
                ui = bui[rows, cl]
                for k, d in enumerate((1, 2, 4)):
                    a_r, a_i = tab[j, 2 * k], tab[j, 2 * k + 1]
                    sr = pltpu.roll(ur, d, 0)
                    si = pltpu.roll(ui, d, 0)
                    ur, ui = ur + (a_r * sr - a_i * si), ui + (a_r * si + a_i * sr)
                wr, wi = tab[j, 6], tab[j, 7]
                c_r, c_i = carry[2 * j], carry[2 * j + 1]
                ur, ui = ur + (wr * c_r - wi * c_i), ui + (wr * c_i + wi * c_r)
                bur[rows, cl] = ur
                bui[rows, cl] = ui
                carry[2 * j] = jnp.broadcast_to(ur[7:8, :], (8, 128))
                carry[2 * j + 1] = jnp.broadcast_to(ui[7:8, :], (8, 128))
        for i in range(2 * NLT):
            hc[i] = carry[i]

    def attn_step(sa, ma, ha, qba, sb, mb, hb, qbb, do_b=True):
        cola = pl.ds(pl.multiple_of(qba * CN, CN), CN)
        q = qT[pl.ds(pl.multiple_of(ha * DH, DH), DH), cola]
        m8 = jnp.full((8, CN), -jnp.inf, F32)
        if do_b:
            tstep = qbb * H + hb
            colb = pl.ds(pl.multiple_of(qbb * CN, CN), CN)
            m = jnp.max(mb[...], axis=0, keepdims=True)
            l8r[...] = jnp.zeros((8, CN), F32)
            acc = jnp.zeros((DH, CN), F32)
        for r in range(NR):
            rows = slice(r * RT, (r + 1) * RT)
            if do_b:
                st = sb[rows, :]
            s = _dot(kS[rows, :], q, 1, 0)
            sa[rows, :] = s
            m8 = jnp.maximum(m8, jnp.max(s.reshape(RT // 8, 8, CN), axis=0))
            if do_b:
                p = jnp.exp(st - m)
                l8r[...] = l8r[...] + jnp.sum(p.reshape(RT // 8, 8, CN), axis=0)
                acc = acc + _dot(vT[:, rows], p.astype(BF16), 1, 0)
                if r in SCAN_AT:
                    scan_blocks(tstep * SPB + SCAN_AT.index(r), 1)
        ma[...] = m8
        if do_b:
            l = jnp.sum(l8r[...], axis=0, keepdims=True)
            oT[pl.ds(pl.multiple_of(hb * DH, DH), DH), colb] = (acc / l).astype(BF16)

    @pl.when(qb == 0)
    def _prologue():
        x = x_ref[...]
        qT[...] = (_dot(wq_ref[...], x, 0, 1) * (DH ** -0.5)).astype(BF16)
        wkv = wkv_ref[...]
        kS[...] = _dot(x, wkv[:, :DH], 1, 0).astype(BF16)
        vT[...] = _dot(wkv[:, DH:], x, 0, 1).astype(BF16)
        gw = _row(gw_ref)
        for rb in range(S // RB):
            rows = slice(rb * RB, (rb + 1) * RB)
            gl = jnp.sum(x_ref[rows, :].astype(F32) * gw, axis=-1, keepdims=True)
            gbuf[rows, :] = jnp.broadcast_to(jax.nn.sigmoid(gl), (RB, 128))

        lre = _row(lre_ref)
        lim = _row(lim_ref)
        dt = jnp.exp(_row(ldt_ref))
        zr = dt * lre
        zi = dt * lim
        ez = jnp.exp(zr)
        lbr = ez * jnp.cos(zi)
        lbi = ez * jnp.sin(zi)
        den = lre * lre + lim * lim
        nr = lbr - 1.0
        cr = (nr * lre + lbi * lim) / den
        ci = (lbi * lre - nr * lim) / den
        cre = cre_ref[...].astype(F32)
        cim = cim_ref[...].astype(F32)
        cpr = cre * cr - cim * ci
        cpi = cre * ci + cim * cr
        wyb[...] = jnp.concatenate([(2.0 * cpr).astype(BF16), (-2.0 * cpi).astype(BF16)], axis=1)

        for rb in range(S // RB):
            rows = slice(rb * RB, (rb + 1) * RB)
            xb = x_ref[rows, :]
            bur[rows, :] = _dot(xb, bre_ref[...], 1, 1)
            bui[rows, :] = _dot(xb, bim_ref[...], 1, 1)

        sub = lax.broadcasted_iota(jnp.int32, (8, 128), 0)
        for j in range(NLT):
            cl = slice(j * 128, (j + 1) * 128)
            p1r = jnp.broadcast_to(lbr[:, cl], (8, 128))
            p1i = jnp.broadcast_to(lbi[:, cl], (8, 128))
            p2r, p2i = _cmul(p1r, p1i, p1r, p1i)
            p4r, p4i = _cmul(p2r, p2i, p2r, p2i)
            for k, (d, pr, pi) in enumerate(((1, p1r, p1i), (2, p2r, p2i), (4, p4r, p4i))):
                tab[j, 2 * k] = jnp.where(sub >= d, pr, 0.0)
                tab[j, 2 * k + 1] = jnp.where(sub >= d, pi, 0.0)
            wr = jnp.where(sub == 0, p1r, 0.0)
            wi = jnp.where(sub == 0, p1i, 0.0)
            ar, ai = p1r, p1i
            for t in range(1, 8):
                ar, ai = _cmul(ar, ai, p1r, p1i)
                wr = jnp.where(sub == t, ar, wr)
                wi = jnp.where(sub == t, ai, wi)
            tab[j, 6] = wr
            tab[j, 7] = wi
        hc[...] = jnp.zeros(hc.shape, F32)

        attn_step(s0, m0, 0, 0, None, None, None, None, do_b=False)

    trip1 = jnp.minimum(qb, 0) + 1

    def one(sa, ma, ha, qba, sb, mb, hb, qbb):
        def body(_, c):
            attn_step(sa, ma, ha, qba, sb, mb, hb, qbb)
            return c
        lax.fori_loop(0, trip1, body, 0)

    def pair(i, _):
        h0 = 2 * i
        one(s1, m1, h0 + 1, qb, s0, m0, h0, qb)
        last = h0 + 2 >= H
        h_n = jnp.where(last, 0, h0 + 2)
        qb_n = jnp.minimum(jnp.where(last, qb + 1, qb), NQ - 1)
        one(s0, m0, h_n, qb_n, s1, m1, h0 + 1, qb)
        return 0

    lax.fori_loop(0, H // 2, pair, 0)

    col = pl.ds(pl.multiple_of(qb * CN, CN), CN)
    a = _dot(oT[:, col], wo_ref[...], 0, 0)
    hcat = jnp.concatenate([bur[col, :].astype(BF16), bui[col, :].astype(BF16)], axis=1)
    b = _dot(hcat, wyb[...], 1, 1) + x_ref[col, :].astype(F32) * _row(dsk_ref)
    g = gbuf[col, :]
    g = jnp.concatenate([g] * (D // 128), axis=1)
    out_ref[...] = g * a + (1.0 - g) * b


@jax.jit
def pallas_gated_mix__grouped_kv_mqa__ssm_conv_s5__prompt_kernel(
    A_x: jax.Array,
    A_wq: jax.Array,
    A_wk: jax.Array,
    A_wv: jax.Array,
    A_wo: jax.Array,
    B_x: jax.Array,
    B_Lambda_re: jax.Array,
    B_Lambda_im: jax.Array,
    B_B_re: jax.Array,
    B_B_im: jax.Array,
    B_C_re: jax.Array,
    B_C_im: jax.Array,
    B_log_dt: jax.Array,
    B_Dskip: jax.Array,
    gate_w: jax.Array,
):
    del B_x
    x = A_x.reshape(S, D)
    A_wkv = jnp.concatenate([A_wk, A_wv], axis=1)
    ins = (x, A_wq, A_wkv, A_wo, B_Lambda_re, B_Lambda_im, B_B_re, B_B_im,
           B_C_re, B_C_im, B_log_dt, B_Dskip, gate_w)
    full = lambda a: pl.BlockSpec(a.shape, lambda qb: (0,) * a.ndim)
    out = pl.pallas_call(
        _kernel,
        grid=(NQ,),
        in_specs=[full(a) for a in ins],
        out_specs=pl.BlockSpec((CN, D), lambda qb: (qb, 0)),
        out_shape=jax.ShapeDtypeStruct((S, D), F32),
        scratch_shapes=[
            pltpu.VMEM((H * DH, S), BF16),
            pltpu.VMEM((S, DH), BF16),
            pltpu.VMEM((DH, S), BF16),
            pltpu.VMEM((H * DH, S), BF16),
            pltpu.VMEM((S, CN), F32),
            pltpu.VMEM((S, CN), F32),
            pltpu.VMEM((8, CN), F32),
            pltpu.VMEM((8, CN), F32),
            pltpu.VMEM((S, P), F32),
            pltpu.VMEM((S, P), F32),
            pltpu.VMEM((S, 128), F32),
            pltpu.VMEM((8, CN), F32),
            pltpu.VMEM((NLT, 8, 8, 128), F32),
            pltpu.VMEM((2 * NLT, 8, 128), F32),
            pltpu.VMEM((D, 2 * P), BF16),
        ],
        compiler_params=pltpu.CompilerParams(
            dimension_semantics=("arbitrary",),
            vmem_limit_bytes=100 * 1024 * 1024,
        ),
    )(*ins)
    return out.reshape(1, S, D)
```

```python
import jax
import jax.numpy as jnp
from jax import lax
import jax.experimental.pallas as pl
import jax.experimental.pallas.tpu as pltpu

S = 2048
D = 512
H = 32
DH = 16
P = 512
CN = 512
NQ = S // CN
RT = 128
NR = S // RT
NLT = P // 128
RB = 256
SPB = (S // 8) // (NQ * H)
SCAN_AT = (0, 8)

F32 = jnp.float32
BF16 = jnp.bfloat16


def _dot(a, b, ca, cb):
    return lax.dot_general(a, b, (((ca,), (cb,)), ((), ())), preferred_element_type=F32)


def _cmul(ar, ai, br, bi):
    return ar * br - ai * bi, ar * bi + ai * br


def _row(ref):
    return ref[...].reshape(1, -1).astype(F32)


def _kernel(x_ref, wq_ref, wkv_ref, lre_ref, lim_ref, ldt_ref, dsk_ref, gw_ref,
            wo_hbm, bre_hbm, bim_hbm, cre_hbm, cim_hbm,
            out_ref,
            qT, kS, vT, oT, s0, s1, m0, m1, bur, bui, gbuf, l8r, tab, hc, wyb,
            wo_ref, bre_ref, bim_ref, cre_ref, cim_ref, dsem):
    qb = pl.program_id(0)

    def late(i, src_hbm, dst):
        return pltpu.make_async_copy(src_hbm, dst, dsem.at[i])

    late_copies = [(wo_hbm, wo_ref), (bre_hbm, bre_ref), (bim_hbm, bim_ref), (cre_hbm, cre_ref), (cim_hbm, cim_ref)]

    def scan_blocks(b0, n):
        carry = [hc[i] for i in range(2 * NLT)]
        for bb in range(n):
            rows = pl.ds(pl.multiple_of((b0 + bb) * 8, 8), 8)
            for j in range(NLT):
                cl = slice(j * 128, (j + 1) * 128)
                ur = bur[rows, cl]
                ui = bui[rows, cl]
                for k, d in enumerate((1, 2, 4)):
                    a_r, a_i = tab[j, 2 * k], tab[j, 2 * k + 1]
                    sr = pltpu.roll(ur, d, 0)
                    si = pltpu.roll(ui, d, 0)
                    ur, ui = ur + (a_r * sr - a_i * si), ui + (a_r * si + a_i * sr)
                wr, wi = tab[j, 6], tab[j, 7]
                c_r, c_i = carry[2 * j], carry[2 * j + 1]
                ur, ui = ur + (wr * c_r - wi * c_i), ui + (wr * c_i + wi * c_r)
                bur[rows, cl] = ur
                bui[rows, cl] = ui
                carry[2 * j] = jnp.broadcast_to(ur[7:8, :], (8, 128))
                carry[2 * j + 1] = jnp.broadcast_to(ui[7:8, :], (8, 128))
        for i in range(2 * NLT):
            hc[i] = carry[i]

    def attn_step(sa, ma, ha, qba, sb, mb, hb, qbb, do_b=True):
        cola = pl.ds(pl.multiple_of(qba * CN, CN), CN)
        q = qT[pl.ds(pl.multiple_of(ha * DH, DH), DH), cola]
        m8 = jnp.full((8, CN), -jnp.inf, F32)
        if do_b:
            tstep = qbb * H + hb
            colb = pl.ds(pl.multiple_of(qbb * CN, CN), CN)
            m = jnp.max(mb[...], axis=0, keepdims=True)
            l8r[...] = jnp.zeros((8, CN), F32)
            acc = jnp.zeros((DH, CN), F32)
        for r in range(NR):
            rows = slice(r * RT, (r + 1) * RT)
            if do_b:
                st = sb[rows, :]
            s = _dot(kS[rows, :], q, 1, 0)
            sa[rows, :] = s
            m8 = jnp.maximum(m8, jnp.max(s.reshape(RT // 8, 8, CN), axis=0))
            if do_b:
                p = jnp.exp(st - m)
                l8r[...] = l8r[...] + jnp.sum(p.reshape(RT // 8, 8, CN), axis=0)
                acc = acc + _dot(vT[:, rows], p.astype(BF16), 1, 0)
                if r in SCAN_AT:
                    scan_blocks(tstep * SPB + SCAN_AT.index(r), 1)
        ma[...] = m8
        if do_b:
            l = jnp.sum(l8r[...], axis=0, keepdims=True)
            oT[pl.ds(pl.multiple_of(hb * DH, DH), DH), colb] = (acc / l).astype(BF16)

    @pl.when(qb == 0)
    def _prologue():
        for i, (src_hbm, dst) in enumerate(late_copies):
            late(i, src_hbm, dst).start()
        x = x_ref[...]
        qT[...] = (_dot(wq_ref[...], x, 0, 1) * (DH ** -0.5)).astype(BF16)
        wkv = wkv_ref[...]
        kS[...] = _dot(x, wkv[:, :DH], 1, 0).astype(BF16)
        vT[...] = _dot(wkv[:, DH:], x, 0, 1).astype(BF16)
        gw = _row(gw_ref)
        for rb in range(S // RB):
            rows = slice(rb * RB, (rb + 1) * RB)
            gl = jnp.sum(x_ref[rows, :].astype(F32) * gw, axis=-1, keepdims=True)
            gbuf[rows, :] = jnp.broadcast_to(jax.nn.sigmoid(gl), (RB, 128))

        lre = _row(lre_ref)
        lim = _row(lim_ref)
        dt = jnp.exp(_row(ldt_ref))
        zr = dt * lre
        zi = dt * lim
        ez = jnp.exp(zr)
        lbr = ez * jnp.cos(zi)
        lbi = ez * jnp.sin(zi)
        den = lre * lre + lim * lim
        nr = lbr - 1.0
        cr = (nr * lre + lbi * lim) / den
        ci = (lbi * lre - nr * lim) / den
        late(3, cre_hbm, cre_ref).wait()
        late(4, cim_hbm, cim_ref).wait()
        cre = cre_ref[...].astype(F32)
        cim = cim_ref[...].astype(F32)
        cpr = cre * cr - cim * ci
        cpi = cre * ci + cim * cr
        wyb[...] = jnp.concatenate([(2.0 * cpr).astype(BF16), (-2.0 * cpi).astype(BF16)], axis=1)

        late(1, bre_hbm, bre_ref).wait()
        late(2, bim_hbm, bim_ref).wait()
        for rb in range(S // RB):
            rows = slice(rb * RB, (rb + 1) * RB)
            xb = x_ref[rows, :]
            bur[rows, :] = _dot(xb, bre_ref[...], 1, 1)
            bui[rows, :] = _dot(xb, bim_ref[...], 1, 1)

        sub = lax.broadcasted_iota(jnp.int32, (8, 128), 0)
        for j in range(NLT):
            cl = slice(j * 128, (j + 1) * 128)
            p1r = jnp.broadcast_to(lbr[:, cl], (8, 128))
            p1i = jnp.broadcast_to(lbi[:, cl], (8, 128))
            p2r, p2i = _cmul(p1r, p1i, p1r, p1i)
            p4r, p4i = _cmul(p2r, p2i, p2r, p2i)
            for k, (d, pr, pi) in enumerate(((1, p1r, p1i), (2, p2r, p2i), (4, p4r, p4i))):
                tab[j, 2 * k] = jnp.where(sub >= d, pr, 0.0)
                tab[j, 2 * k + 1] = jnp.where(sub >= d, pi, 0.0)
            wr = jnp.where(sub == 0, p1r, 0.0)
            wi = jnp.where(sub == 0, p1i, 0.0)
            ar, ai = p1r, p1i
            for t in range(1, 8):
                ar, ai = _cmul(ar, ai, p1r, p1i)
                wr = jnp.where(sub == t, ar, wr)
                wi = jnp.where(sub == t, ai, wi)
            tab[j, 6] = wr
            tab[j, 7] = wi
        hc[...] = jnp.zeros(hc.shape, F32)

        attn_step(s0, m0, 0, 0, None, None, None, None, do_b=False)

    trip1 = jnp.minimum(qb, 0) + 1

    def one(sa, ma, ha, qba, sb, mb, hb, qbb):
        def body(_, c):
            attn_step(sa, ma, ha, qba, sb, mb, hb, qbb)
            return c
        lax.fori_loop(0, trip1, body, 0)

    def pair(i, _):
        h0 = 2 * i
        one(s1, m1, h0 + 1, qb, s0, m0, h0, qb)
        last = h0 + 2 >= H
        h_n = jnp.where(last, 0, h0 + 2)
        qb_n = jnp.minimum(jnp.where(last, qb + 1, qb), NQ - 1)
        one(s0, m0, h_n, qb_n, s1, m1, h0 + 1, qb)
        return 0

    lax.fori_loop(0, H // 2, pair, 0)

    @pl.when(qb == 0)
    def _():
        late(0, wo_hbm, wo_ref).wait()

    col = pl.ds(pl.multiple_of(qb * CN, CN), CN)
    a = _dot(oT[:, col], wo_ref[...], 0, 0)
    hcat = jnp.concatenate([bur[col, :].astype(BF16), bui[col, :].astype(BF16)], axis=1)
    b = _dot(hcat, wyb[...], 1, 1) + x_ref[col, :].astype(F32) * _row(dsk_ref)
    g = gbuf[col, :]
    g = jnp.concatenate([g] * (D // 128), axis=1)
    out_ref[...] = g * a + (1.0 - g) * b


@jax.jit
def pallas_gated_mix__grouped_kv_mqa__ssm_conv_s5__prompt_kernel(
    A_x: jax.Array,
    A_wq: jax.Array,
    A_wk: jax.Array,
    A_wv: jax.Array,
    A_wo: jax.Array,
    B_x: jax.Array,
    B_Lambda_re: jax.Array,
    B_Lambda_im: jax.Array,
    B_B_re: jax.Array,
    B_B_im: jax.Array,
    B_C_re: jax.Array,
    B_C_im: jax.Array,
    B_log_dt: jax.Array,
    B_Dskip: jax.Array,
    gate_w: jax.Array,
):
    del B_x
    x = A_x.reshape(S, D)
    A_wkv = jnp.concatenate([A_wk, A_wv], axis=1)
    early = (x, A_wq, A_wkv, B_Lambda_re, B_Lambda_im, B_log_dt, B_Dskip, gate_w)
    late_in = (A_wo, B_B_re, B_B_im, B_C_re, B_C_im)
    ins = early + late_in
    full = lambda a: pl.BlockSpec(a.shape, lambda qb: (0,) * a.ndim)
    out = pl.pallas_call(
        _kernel,
        grid=(NQ,),
        in_specs=[full(a) for a in early] + [pl.BlockSpec(memory_space=pl.ANY) for _ in late_in],
        out_specs=pl.BlockSpec((CN, D), lambda qb: (qb, 0)),
        out_shape=jax.ShapeDtypeStruct((S, D), F32),
        scratch_shapes=[
            pltpu.VMEM((H * DH, S), BF16),
            pltpu.VMEM((S, DH), BF16),
            pltpu.VMEM((DH, S), BF16),
            pltpu.VMEM((H * DH, S), BF16),
            pltpu.VMEM((S, CN), F32),
            pltpu.VMEM((S, CN), F32),
            pltpu.VMEM((8, CN), F32),
            pltpu.VMEM((8, CN), F32),
            pltpu.VMEM((S, P), F32),
            pltpu.VMEM((S, P), F32),
            pltpu.VMEM((S, 128), F32),
            pltpu.VMEM((8, CN), F32),
            pltpu.VMEM((NLT, 8, 8, 128), F32),
            pltpu.VMEM((2 * NLT, 8, 128), F32),
            pltpu.VMEM((D, 2 * P), BF16),
            pltpu.VMEM(A_wo.shape, BF16),
            pltpu.VMEM(B_B_re.shape, BF16),
            pltpu.VMEM(B_B_im.shape, BF16),
            pltpu.VMEM(B_C_re.shape, BF16),
            pltpu.VMEM(B_C_im.shape, BF16),
            pltpu.SemaphoreType.DMA((5,)),
        ],
        compiler_params=pltpu.CompilerParams(
            dimension_semantics=("arbitrary",),
            vmem_limit_bytes=100 * 1024 * 1024,
        ),
    )(*ins)
    return out.reshape(1, S, D)
```
